```python
import os as _os
_os.environ.setdefault('JAX_PLATFORMS', 'cpu')
import jax
import jax.numpy as jnp

def _softmax(x, axis=-1):
    return jax.nn.softmax(x, axis=axis)

def _gelu(x):
    return jax.nn.gelu(x, approximate=True)

def _silu(x):
    return jax.nn.silu(x)

def _sigmoid(x):
    return jax.nn.sigmoid(x)

def _layernorm(x, axis=-1, eps=1e-05):
    m = jnp.mean(x, axis=axis, keepdims=True)
    v = jnp.var(x, axis=axis, keepdims=True)
    return (x - m) / jnp.sqrt(v + eps)

def _scatter_add(tgt, idx, src, axis=0):
    return tgt.at[idx].add(src)

def _segment_sum(src, seg, n):
    return jax.ops.segment_sum(src, seg, n)

class _Rng:

    def __init__(self, key):
        self._k = key

    def _next(self):
        self._k, sub = jax.random.split(self._k)
        return sub

    def normal(self, shape):
        return jax.random.normal(self._next(), shape, dtype=jnp.bfloat16)

    def randint(self, lo, hi, shape):
        return jax.random.randint(self._next(), shape, lo, hi, dtype=jnp.int32)

    def uniform(self, shape, lo=0.0, hi=1.0):
        return jax.random.uniform(self._next(), shape, jnp.bfloat16, lo, hi)

    def permutation(self, n):
        return jax.random.permutation(self._next(), n)
kernel_name = 'standalone__conformer_conv_module__speech'

def setup_inputs():
    _rng = _Rng(jax.random.key(int.from_bytes(__import__("os").urandom(4), "little")))
    _w = lambda a: (lambda t: t.astype(jnp.bfloat16) if jnp.issubdtype(t.dtype, jnp.floating) else t)(jnp.asarray(a))
    B, T, D, K = (2, 16000, 256, 5)
    return {'x': _w((lambda *s: _rng.normal(s) * 0.2)(B, T, D)), 'w_pw1': _w((lambda *s: _rng.normal(s) * 0.2)(D, 2 * D)), 'dw': _w((lambda *s: _rng.normal(s) * 0.05)(K, D)), 'w_pw2': _w((lambda *s: _rng.normal(s) * 0.05)(D, D))}

def reference(x, w_pw1, dw, w_pw2):
    B, T, D = x.shape
    K = dw.shape[0]
    h = x @ w_pw1
    a, b = (h[..., :D].copy(), h[..., D:].copy())
    h = a * _sigmoid(b)
    pad = K // 2
    hp = jnp.pad(h, ((0, 0), (pad, pad), (0, 0)))
    out = jnp.zeros_like(h)
    for i in range(K):
        out = out + hp[:, i:i + T, :] * dw[i][None, None, :]
    return _silu(out) @ w_pw2
```

```python
import functools
import jax
import jax.numpy as jnp
import jax.experimental.pallas as pl
import jax.experimental.pallas.tpu as pltpu

TT = 4000
HALO = 16
FIRST = (320, 1120, 2560)
LAST = (2400, 960, 400, 240)
PRI = 1
NOCHECK = False

def _kernel(x_hbm, w1_hbm, dw_hbm, w2_hbm, o_hbm,
            xbuf, obuf, h_scr, w1_v, dw_v, w2_v, w1s, isem, osem, wsem, fsem, lsem, *, D, K, T, BT):
    H = D // 2
    ns = BT // TT
    XR = TT + 2 * HALO

    w_cps = [pltpu.make_async_copy(w1_hbm, w1_v, wsem.at[0]),
             pltpu.make_async_copy(dw_hbm, dw_v, wsem.at[1]),
             pltpu.make_async_copy(w2_hbm, w2_v, wsem.at[2])]

    def first_in(j):
        lo = sum(FIRST[:j])
        n = FIRST[j] + (HALO if j == len(FIRST) - 1 else 0)
        return pltpu.make_async_copy(x_hbm.at[pl.ds(lo, n), :], xbuf.at[0, pl.ds(HALO + lo, n), :], fsem.at[j])

    def in_copy(s, slot):
        st = jnp.minimum(s * TT - HALO, BT - XR)
        return pltpu.make_async_copy(x_hbm.at[pl.ds(pl.multiple_of(st, HALO), XR), :], xbuf.at[slot], isem.at[slot])

    def out_copy(s, slot):
        return pltpu.make_async_copy(obuf.at[slot], o_hbm.at[pl.ds(pl.multiple_of(s * TT, HALO), TT), :], osem.at[slot])

    def last_out(j):
        lo = sum(LAST[:j])
        slot = (ns - 1) % 2
        return pltpu.make_async_copy(obuf.at[slot, pl.ds(lo, LAST[j]), :],
                                     o_hbm.at[pl.ds((ns - 1) * TT + lo, LAST[j]), :], lsem.at[j])

    def stage1(slot, xlo, hlo, n, lead_valid, trail_valid):
        xa = xbuf[slot, pl.ds(xlo, n), :]
        for c in range(2):
            hh = jnp.dot(xa, w1s[c], preferred_element_type=jnp.float32)
            a = hh[:, :H]
            h = a * jnp.tanh(hh[:, H:]) + a
            valid = None
            if lead_valid is not None or trail_valid is not None:
                rows = jax.lax.broadcasted_iota(jnp.int32, (n, 1), 0)
                if lead_valid is not None:
                    valid = jnp.logical_or(rows >= HALO, lead_valid)
                if trail_valid is not None:
                    v2 = jnp.logical_or(rows < n - HALO, trail_valid)
                    valid = v2 if valid is None else jnp.logical_and(valid, v2)
                h = jnp.where(valid, h, 0.0)
            h_scr[c, pl.ds(hlo, n), :] = h

    def stage2(slot, lo, n):
        dw = dw_v[...].astype(jnp.float32) * 0.5
        gs = []
        for c in range(2):
            dwc = dw[:, c * H:(c + 1) * H]
            base = HALO - 2 + lo
            u = h_scr[c, pl.ds(base, n), :] * dwc[0:1, :]
            for k in range(1, K):
                u = u + h_scr[c, pl.ds(base + k, n), :] * dwc[k:k + 1, :]
            g = u * jnp.tanh(u) + u
            gs.append(g.astype(jnp.bfloat16))
        g = jnp.concatenate(gs, axis=1)
        obuf[slot, pl.ds(lo, n), :] = jnp.dot(g, w2_v[...], preferred_element_type=jnp.float32).astype(obuf.dtype)

    def lead_ok(s):
        return (s * TT) % T != 0

    def trail_ok(s):
        return ((s + 1) * TT) % T != 0

    w_cps[0].start()
    first_in(0).start()
    w_cps[2].start()
    w_cps[1].start()
    for j in range(1, len(FIRST)):
        first_in(j).start(priority=PRI)
    in_copy(1, 1).start(priority=PRI)
    w_cps[0].wait()
    for c in range(2):
        w = jnp.concatenate([w1_v[:, c * H:(c + 1) * H], w1_v[:, D + c * H:D + (c + 1) * H]], axis=1)
        w1s[c] = (w.astype(jnp.float32) * 0.5).astype(jnp.bfloat16)
    h_scr[:, pl.ds(0, HALO), :] = jnp.zeros((2, HALO, H), jnp.float32)
    nf = len(FIRST)
    done2 = 0
    for j in range(nf):
        first_in(j).wait()
        if j == 0:
            w_cps[1].wait()
            w_cps[2].wait()
        lo = sum(FIRST[:j])
        last = j == nf - 1
        n = FIRST[j] + (HALO if last else 0)
        stage1(0, HALO + lo, HALO + lo, n, None, trail_ok(0) if last else None)
        hi = lo + FIRST[j] - (0 if last else HALO)
        stage2(0, done2, hi - done2)
        done2 = hi
    out_copy(0, 0).start()

    def body(s, carry):
        slot = s % 2
        @pl.when(s >= 2)
        def _():
            out_copy(s - 2, slot).wait()

        in_copy(s, slot).wait()
        in_copy(s + 1, 1 - slot).start()
        stage1(slot, 0, 0, XR, lead_ok(s), trail_ok(s))
        stage2(slot, 0, TT)
        out_copy(s, slot).start()
        return carry

    jax.lax.fori_loop(1, ns - 1, body, 0)

    s = ns - 1
    slot = s % 2
    out_copy(s - 2, slot).wait()
    in_copy(s, slot).wait()
    h_scr[:, pl.ds(HALO + TT, HALO), :] = jnp.zeros((2, HALO, H), jnp.float32)
    nl = len(LAST)
    done1 = 0
    for j in range(nl):
        need = min(HALO + sum(LAST[:j + 1]) + HALO, HALO + TT)
        stage1(slot, HALO + done1, done1, need - done1, lead_ok(s) if j == 0 else None, None)
        done1 = need
        stage2(slot, sum(LAST[:j]), LAST[j])
        last_out(j).start()
    out_copy(s - 1, 1 - slot).wait()
    for j in range(len(LAST)):
        last_out(j).wait()


@jax.jit
def pallas_standalone__conformer_conv_module__speech_kernel(x, w_pw1, dw, w_pw2):
    B, T, D = x.shape
    K = dw.shape[0]
    BT = B * T
    out = pl.pallas_call(
        functools.partial(_kernel, D=D, K=K, T=T, BT=BT),
        in_specs=[pl.BlockSpec(memory_space=pl.ANY)] * 4,
        out_specs=pl.BlockSpec(memory_space=pl.ANY),
        out_shape=jax.ShapeDtypeStruct((BT, D), x.dtype),
        scratch_shapes=[
            pltpu.VMEM((2, TT + 2 * HALO, D), jnp.bfloat16),
            pltpu.VMEM((2, TT, D), jnp.bfloat16),
            pltpu.VMEM((2, TT + 2 * HALO, D // 2), jnp.float32),
            pltpu.VMEM((D, 2 * D), jnp.bfloat16),
            pltpu.VMEM((K, D), jnp.bfloat16),
            pltpu.VMEM((D, D), jnp.bfloat16),
            pltpu.VMEM((2, D, D), jnp.bfloat16),
            pltpu.SemaphoreType.DMA((2,)),
            pltpu.SemaphoreType.DMA((2,)),
            pltpu.SemaphoreType.DMA((3,)),
            pltpu.SemaphoreType.DMA((len(FIRST),)),
            pltpu.SemaphoreType.DMA((len(LAST),)),
        ],
        compiler_params=pltpu.CompilerParams(
            vmem_limit_bytes=100 * 1024 * 1024,
            disable_bounds_checks=NOCHECK),
    )(x.reshape(BT, D), w_pw1, dw, w_pw2)
    return out.reshape(B, T, D)
```

```python
import functools

import jax
import jax.numpy as jnp
import jax.experimental.pallas as pl
import jax.experimental.pallas.tpu as pltpu

HALO = 16
FIRST = (320, 1120, 2560)
LAST = (2400, 960, 400, 240)
TM = 6000
TF = sum(FIRST)
TL = sum(LAST)


def _kernel(x_hbm, w1_hbm, dw_hbm, w2_hbm, o_hbm,
            xbuf, obuf, h_scr, carry, w1_v, dw_v, w2_v, w1s,
            isem, osem, wsem, fsem, lsem, *, D, K, T, BT):
    H = D // 2
    nm = (BT - TF - TL) // TM
    assert TF + nm * TM + TL == BT and (T - TF) % TM == 0 and nm >= 2 and TL <= TM
    assert K // 2 <= HALO and BT == 2 * T
    RL = BT - TL
    lslot = (nm + 1) % 2

    def r0(m):
        return TF + m * TM

    w_cps = [pltpu.make_async_copy(w1_hbm, w1_v, wsem.at[0]),
             pltpu.make_async_copy(dw_hbm, dw_v, wsem.at[1]),
             pltpu.make_async_copy(w2_hbm, w2_v, wsem.at[2])]

    def first_in(j):
        lo = sum(FIRST[:j])
        n = FIRST[j] + (HALO if j == len(FIRST) - 1 else 0)
        return pltpu.make_async_copy(x_hbm.at[pl.ds(lo, n), :], xbuf.at[0, pl.ds(lo, n), :], fsem.at[j])

    def in_copy(m, slot):
        st = jnp.minimum(r0(m) + HALO, BT - TM)
        return pltpu.make_async_copy(x_hbm.at[pl.ds(pl.multiple_of(st, HALO), TM), :],
                                     xbuf.at[slot, pl.ds(0, TM), :], isem.at[slot])

    def out_copy(m, slot):
        return pltpu.make_async_copy(obuf.at[slot, pl.ds(0, TM), :],
                                     o_hbm.at[pl.ds(pl.multiple_of(r0(m), HALO), TM), :], osem.at[slot])

    first_out = pltpu.make_async_copy(obuf.at[0, pl.ds(0, TF), :], o_hbm.at[pl.ds(0, TF), :], osem.at[2])

    def last_out(j):
        lo = sum(LAST[:j])
        return pltpu.make_async_copy(obuf.at[lslot, pl.ds(lo, LAST[j]), :],
                                     o_hbm.at[pl.ds(RL + lo, LAST[j]), :], lsem.at[j])

    def stage1(slot, xlo, hlo, n, trail_valid):
        xa = xbuf[slot, pl.ds(xlo, n), :]
        for c in range(2):
            hh = jnp.dot(xa, w1s[c], preferred_element_type=jnp.float32)
            a = hh[:, :H]
            h = a * jnp.tanh(hh[:, H:]) + a
            if trail_valid is not None:
                carry[c] = h[n - 2 * HALO:, :]
                h_scr[c, pl.ds(hlo, n - HALO), :] = h[:n - HALO, :]
                h_scr[c, pl.ds(hlo + n - HALO, HALO), :] = jnp.where(trail_valid, h[n - HALO:, :], 0.0)
            else:
                h_scr[c, pl.ds(hlo, n), :] = h

    def load_carry(lead_valid):
        for c in range(2):
            cv = carry[c]
            h_scr[c, pl.ds(0, HALO), :] = jnp.where(lead_valid, cv[:HALO, :], 0.0)
            h_scr[c, pl.ds(HALO, HALO), :] = cv[HALO:, :]

    def stage2(slot, lo, n):
        dw = dw_v[...].astype(jnp.float32) * 0.5
        gs = []
        for c in range(2):
            dwc = dw[:, c * H:(c + 1) * H]
            base = HALO - K // 2 + lo
            u = h_scr[c, pl.ds(base, n), :] * dwc[0:1, :]
            for k in range(1, K):
                u = u + h_scr[c, pl.ds(base + k, n), :] * dwc[k:k + 1, :]
            g = u * jnp.tanh(u) + u
            gs.append(g.astype(jnp.bfloat16))
        g = jnp.concatenate(gs, axis=1)
        obuf[slot, pl.ds(lo, n), :] = jnp.dot(
            g, w2_v[...], preferred_element_type=jnp.float32).astype(obuf.dtype)

    w_cps[0].start()
    first_in(0).start()
    w_cps[2].start()
    w_cps[1].start()
    for j in range(1, len(FIRST)):
        first_in(j).start(priority=1)
    in_copy(0, 1).start(priority=1)

    w_cps[0].wait()
    for c in range(2):
        w = jnp.concatenate([w1_v[:, c * H:(c + 1) * H], w1_v[:, D + c * H:D + (c + 1) * H]], axis=1)
        w1s[c] = (w.astype(jnp.float32) * 0.5).astype(jnp.bfloat16)
    h_scr[:, pl.ds(0, HALO), :] = jnp.zeros((2, HALO, H), jnp.float32)
    done2 = 0
    for j in range(len(FIRST)):
        first_in(j).wait()
        if j == 0:
            w_cps[1].wait()
            w_cps[2].wait()
        lo = sum(FIRST[:j])
        last = j == len(FIRST) - 1
        stage1(0, lo, HALO + lo, FIRST[j] + (HALO if last else 0), (TF % T != 0) if last else None)
        hi = lo + FIRST[j] - (0 if last else HALO)
        stage2(0, done2, hi - done2)
        done2 = hi
    first_out.start()

    def body(m, unused):
        slot = (m + 1) % 2

        @pl.when(m == 1)
        def _():
            first_out.wait()

        @pl.when(m >= 2)
        def _():
            out_copy(m - 2, slot).wait()

        in_copy(m, slot).wait()
        in_copy(m + 1, 1 - slot).start()
        load_carry(r0(m) % T != 0)
        stage1(slot, 0, 2 * HALO, TM, (r0(m) + TM) % T != 0)
        stage2(slot, 0, TM)
        out_copy(m, slot).start()
        return unused

    jax.lax.fori_loop(0, nm, body, 0)

    out_copy(nm - 2, lslot).wait()
    in_copy(nm, lslot).wait()
    load_carry(RL % T != 0)
    h_scr[:, pl.ds(HALO + TL, HALO), :] = jnp.zeros((2, HALO, H), jnp.float32)
    xoff = TM - TL
    done1 = 2 * HALO
    for j in range(len(LAST)):
        need = min(2 * HALO + sum(LAST[:j + 1]), HALO + TL)
        stage1(lslot, xoff + done1 - HALO, done1, need - done1, None)
        done1 = need
        stage2(lslot, sum(LAST[:j]), LAST[j])
        last_out(j).start()
    out_copy(nm - 1, 1 - lslot).wait()
    for j in range(len(LAST)):
        last_out(j).wait()


@jax.jit
def pallas_standalone__conformer_conv_module__speech_kernel(
    x: jax.Array,
    w_pw1: jax.Array,
    dw: jax.Array,
    w_pw2: jax.Array,
):
    B, T, D = x.shape
    K = dw.shape[0]
    BT = B * T
    R = max(TF, TM, TL)
    out = pl.pallas_call(
        functools.partial(_kernel, D=D, K=K, T=T, BT=BT),
        in_specs=[pl.BlockSpec(memory_space=pl.ANY)] * 4,
        out_specs=pl.BlockSpec(memory_space=pl.ANY),
        out_shape=jax.ShapeDtypeStruct((BT, D), x.dtype),
        scratch_shapes=[
            pltpu.VMEM((2, R + HALO, D), jnp.bfloat16),
            pltpu.VMEM((2, R, D), jnp.bfloat16),
            pltpu.VMEM((2, R + 2 * HALO, D // 2), jnp.float32),
            pltpu.VMEM((2, 2 * HALO, D // 2), jnp.float32),
            pltpu.VMEM((D, 2 * D), jnp.bfloat16),
            pltpu.VMEM((K, D), jnp.bfloat16),
            pltpu.VMEM((D, D), jnp.bfloat16),
            pltpu.VMEM((2, D, D), jnp.bfloat16),
            pltpu.SemaphoreType.DMA((2,)),
            pltpu.SemaphoreType.DMA((3,)),
            pltpu.SemaphoreType.DMA((3,)),
            pltpu.SemaphoreType.DMA((len(FIRST),)),
            pltpu.SemaphoreType.DMA((len(LAST),)),
        ],
        compiler_params=pltpu.CompilerParams(vmem_limit_bytes=100 * 1024 * 1024),
    )(x.reshape(BT, D), w_pw1, dw, w_pw2)
    return out.reshape(B, T, D)
```
